```python
import os as _os
_os.environ.setdefault("JAX_PLATFORMS", "cpu")
import jax
import jax.numpy as jnp

def _softmax(x, axis=-1):
    return jax.nn.softmax(x, axis=axis)
def _gelu(x):
    return jax.nn.gelu(x, approximate=True)
def _silu(x):
    return jax.nn.silu(x)
def _sigmoid(x):
    return jax.nn.sigmoid(x)
def _layernorm(x, axis=-1, eps=1e-5):
    m = jnp.mean(x, axis=axis, keepdims=True)
    v = jnp.var(x, axis=axis, keepdims=True)
    return (x - m) / jnp.sqrt(v + eps)
def _scatter_add(tgt, idx, src, axis=0):
    return tgt.at[idx].add(src)
def _segment_sum(src, seg, n):
    return jax.ops.segment_sum(src, seg, n)
class _Rng:
    def __init__(self, key):
        self._k = key
    def _next(self):
        self._k, sub = jax.random.split(self._k)
        return sub
    def normal(self, shape):
        return jax.random.normal(self._next(), shape, dtype=jnp.bfloat16)
    def randint(self, lo, hi, shape):
        return jax.random.randint(self._next(), shape, lo, hi, dtype=jnp.int32)
    def uniform(self, shape, lo=0.0, hi=1.0):
        return jax.random.uniform(self._next(), shape, jnp.bfloat16, lo, hi)
    def permutation(self, n):
        return jax.random.permutation(self._next(), n)


kernel_name = 'sequential_preLN__mha_block__moe_arch_mod__prompt'

def setup_inputs():
    _rng = _Rng(jax.random.key(int.from_bytes(__import__("os").urandom(4), "little")))
    _w = (lambda a: (lambda t: t.astype(jnp.bfloat16) if jnp.issubdtype(t.dtype, jnp.floating) else t)(jnp.asarray(a)))
    def _A_setup():
        B, S, D, H = 1, 2048, 640, 32
        return {
            "x": _w((lambda *s: _rng.normal(s) * 0.05)(B, S, D)),
            "wqkv": _w((lambda *s: _rng.normal(s) * 0.05)(D, 3 * D)),
            "wo": _w((lambda *s: _rng.normal(s) * 0.05)(D, D)),
        }
    _A_in = _A_setup()

    def _B_setup():
        B, S, D, F, C = 1, 2048, 640, 1536, 1
        return {
            "x": _w((lambda *s: _rng.normal(s) * 0.05)(B, S, D)),
            "w_r": _w((lambda *s: _rng.normal(s) * 0.05)(D)),
            "w_gate": _w((lambda *s: _rng.normal(s) * 0.05)(D, F)),
            "w_up": _w((lambda *s: _rng.normal(s) * 0.05)(D, F)),
            "w_down": _w((lambda *s: _rng.normal(s) * 0.05)(F, D)),
        }
    _B_in = _B_setup()

    return {
        "A_x": _A_in["x"],
        "A_wqkv": _A_in["wqkv"],
        "A_wo": _A_in["wo"],
        "B_x": _B_in["x"],
        "B_w_r": _B_in["w_r"],
        "B_w_gate": _B_in["w_gate"],
        "B_w_up": _B_in["w_up"],
        "B_w_down": _B_in["w_down"],
    }

def reference(A_x, A_wqkv, A_wo, B_x, B_w_r, B_w_gate, B_w_up, B_w_down):
    def _A_ref(x, wqkv, wo):
        B, S, D = x.shape
        H = 32
        Dh = D // H
        qkv = (lambda x, *d: x.transpose(*d))((x @ wqkv).reshape(B, S, 3, H, Dh), 2, 0, 3, 1, 4)
        q, k, v = qkv[0], qkv[1], qkv[2]
        scores = jnp.einsum("bhqd,bhkd->bhqk", q, k) * (Dh ** -0.5)
        p = _softmax(scores, axis=-1)
        o = jnp.einsum("bhqk,bhkd->bhqd", p, v)
        return (lambda x, *d: x.transpose(*d))(o, 0, 2, 1, 3).reshape(B, S, D) @ wo

    def _B_ref(x, w_r, w_gate, w_up, w_down):
        B, S, D = x.shape
        C = 1
        r = x @ w_r
        idx = jnp.argsort(-r, axis=-1)[:, :C]
        idx_e = jnp.repeat(idx.reshape(B, C, 1), D, axis=2)
        x_sel = jnp.take_along_axis(x, idx_e, axis=1)
        g = _silu(x_sel @ w_gate)
        u = x_sel @ w_up
        y = (g * u) @ w_down
        r_sel = _sigmoid(jnp.take_along_axis(r, idx, axis=1))
        y = y * r_sel.reshape(B, C, 1)
        b_off = (jnp.arange(B) * S).reshape(B, 1)
        flat_idx = (idx + b_off).reshape(B * C)
        zero = (x * 0.0).reshape(B * S, D)
        upd = _scatter_add(zero, flat_idx, y.reshape(B * C, D), axis=0)
        return x + upd.reshape(B, S, D)

    x = A_x
    h = x + _A_ref(_layernorm(x, axis=-1), A_wqkv, A_wo)
    h2 = h + _B_ref(_layernorm(h, axis=-1), B_w_r, B_w_gate, B_w_up, B_w_down)
    return h2
```

```python
import jax
import jax.numpy as jnp
from jax import lax
import jax.experimental.pallas as pl
import jax.experimental.pallas.tpu as pltpu

S, D, H, DH, F = 2048, 640, 32, 20, 1536
NT = 19
GP = 108
NG = 5
NV = 9
STRADDLE = (6, 12, 19, 25)
KTR = 344
QSCALE = float(DH ** -0.5 * 1.4426950408889634)
EPS = 1e-5
CH = 512
LP = 128
OCH = 128
U = 2
NCH = 8
RC = S // NCH
GUARD = 2.0 ** 64
f32 = jnp.float32
bf16 = jnp.bfloat16
u32 = jnp.uint32

PIECES = tuple([(b, GP, 20, 16 + b // 5, 20 * (b % 5)) for b in range(15)]
               + [(15, GP, 8, 16, 100), (15, GP + 8, 8, 17, 100), (15, GP + 16, 4, 18, 100)])


def _ln(xf):
    m = jnp.mean(xf, axis=-1, keepdims=True)
    d = xf - m
    v = jnp.mean(d * d, axis=-1, keepdims=True)
    return d * lax.rsqrt(v + EPS)


def _iota(shape, dim):
    return lax.broadcasted_iota(jnp.int32, shape, dim)


def _kernel(x_hbm, wqkv_hbm, wo_hbm, wr_hbm, wg_hbm, wu_hbm, wd_hbm, out_hbm,
            x_v, xn_v, wq_v, wk_v, wv_v, wkt_v, wo_v, wr_v, wg_v, wu_v, wd_v,
            q_v, v_v, kt_v, qh_v, acc_v, l0_v, w0_v, attn_v, h_v, out_v, patch_v,
            top_v, sems, osems):
    NC = S // CH
    xcps = [pltpu.make_async_copy(x_hbm.at[pl.ds(c * CH, CH), :], x_v.at[pl.ds(c * CH, CH), :], sems.at[c])
            for c in range(NC)]
    wq_cp = pltpu.make_async_copy(wqkv_hbm.at[:, pl.ds(0, D)], wq_v, sems.at[NC])
    wv_cp = pltpu.make_async_copy(wqkv_hbm.at[:, pl.ds(2 * D, D)], wv_v, sems.at[NC + 1])
    wk_cp = pltpu.make_async_copy(wqkv_hbm.at[:, pl.ds(D, D)], wk_v, sems.at[NC + 2])
    late = [
        pltpu.make_async_copy(wo_hbm, wo_v, sems.at[NC + 3]),
        pltpu.make_async_copy(wr_hbm, wr_v, sems.at[NC + 4]),
        pltpu.make_async_copy(wg_hbm, wg_v, sems.at[NC + 5]),
        pltpu.make_async_copy(wu_hbm, wu_v, sems.at[NC + 6]),
        pltpu.make_async_copy(wd_hbm, wd_v, sems.at[NC + 7]),
    ]
    xcps[0].start()
    wq_cp.start()
    wv_cp.start()
    wk_cp.start()
    for c in range(1, NC):
        xcps[c].start()

    for t in range(16, NT):
        v_v[:, t * 64:(t + 1) * 64, :] = jnp.zeros((NV, 64, 128), u32)
    for t in range(NT):
        kt_v[t, 0:8, :] = jnp.zeros((8, 128), u32)
        kt_v[t, 328:344, :] = jnp.zeros((16, 128), u32)
    acc_v[...] = jnp.ones((S, 128), f32)

    def head_geom(h):
        if isinstance(h, int):
            return (DH * h) % 128, (NG + STRADDLE.index(h) if h in STRADDLE else (DH * h) // 128)
        c = (DH * h) & 127
        virt = NG + (h >= 12).astype(jnp.int32) + (h >= 19).astype(jnp.int32) + (h >= 25).astype(jnp.int32)
        g = jnp.where(c + DH > 128, virt, lax.shift_right_logical(DH * h, 7))
        return c, g

    lane64 = _iota((64, 128), 1)
    row16 = _iota((16, 128), 0)
    lane16 = _iota((16, 128), 1)
    lane_c = _iota((RC, 128), 1)
    M = {'gap64': lane64 >= GP, 'gap16': lane16 >= GP, 'row16': row16 >= 6, 'gap_c': lane_c >= GP}
    M0 = dict(M)
    zu = jnp.zeros((), u32)

    def w_vpart(h, j):
        c, g = head_geom(h)
        r0 = pl.multiple_of(j * 64, 64)
        vt = pltpu.roll(v_v[g, pl.ds(r0, 64), :], (GP - c + 128) & 127, 1)
        return jnp.where(M['gap64'], vt, zu)

    def w_kwin(h, j):
        return kt_v[j, pl.ds(10 * h + 2, 16), :]

    def build_w(h, jv, hk, jk, raw=False):
        wv = w_vpart(h, jv)
        kw = jnp.where(M['gap16'], zu, w_kwin(hk, jk))
        low = jnp.where(M['row16'], kw, wv[48:64, :])
        wu = jnp.concatenate([wv[0:48, :], low], axis=0)
        return wu if raw else pltpu.bitcast(wu, bf16)

    def build_wk(hk, jk):
        kw = jnp.where((lane16 < GP) & (row16 >= 6), w_kwin(hk, jk), zu)
        return pltpu.bitcast(jnp.concatenate([jnp.zeros((48, 128), u32), kw], axis=0), bf16)

    def build_wv(h, j):
        wv = w_vpart(h, j)
        low = jnp.where(row16 >= 6, zu, wv[48:64, :])
        return pltpu.bitcast(jnp.concatenate([wv[0:48, :], low], axis=0), bf16)

    lane_k = _iota((D // 2, 128), 1)
    lane_p = _iota((CH // 2, 128), 1)
    lane_r = _iota((CH, 128), 1)
    gap_r = lane_r >= GP
    ktiles = {}
    NPC = CH // LP

    def ln_piece(c, p):
        rows = pl.ds(c * CH + p * LP, LP)
        xn_v[rows, :] = _ln(x_v[rows, :].astype(f32)).astype(bf16)

    def proj_q(c, xn):
        rows = pl.ds(c * CH, CH)
        qq = jnp.dot(xn, wq_v[...], preferred_element_type=f32) * QSCALE
        for g in range(NG):
            q_v[g, rows, :] = qq[:, g * 128:(g + 1) * 128]
        for i, hh in enumerate(STRADDLE):
            cc = (DH * hh) % 128
            gg = (DH * hh) // 128
            q_v[NG + i, rows, :] = jnp.where(lane_r >= cc, qq[:, gg * 128:(gg + 1) * 128],
                                             qq[:, (gg + 1) * 128:(gg + 2) * 128])
        qh_v[rows, :] = pltpu.roll(qq[:, 0:128], GP, 1)

    def proj_v(c, xn):
        vv = jnp.dot(xn, wv_v[...], preferred_element_type=f32)
        vv = pltpu.bitcast(vv.astype(bf16), u32)
        prow = pl.ds(c * (CH // 2), CH // 2)
        for g in range(NG):
            v_v[g, prow, :] = vv[:, g * 128:(g + 1) * 128]
        for i, hh in enumerate(STRADDLE):
            cc = (DH * hh) % 128
            gg = (DH * hh) // 128
            v_v[NG + i, prow, :] = jnp.where(lane_p >= cc, vv[:, gg * 128:(gg + 1) * 128],
                                             vv[:, (gg + 1) * 128:(gg + 2) * 128])

    def proj_k(c, xn):
        kt = lax.dot_general(wkt_v[...], xn, (((1,), (1,)), ((), ())), preferred_element_type=f32)
        kt = pltpu.bitcast(kt.astype(bf16), u32)
        for t in range(CH // 128):
            b = c * (CH // 128) + t
            ktb = kt[:, t * 128:(t + 1) * 128]
            kt_v[b, 8:328, :] = ktb
            for (bb, so, n, tt, slot) in PIECES:
                if bb == b:
                    src = pltpu.roll(ktb, (slot - so) % 128, 1)
                    msk = (lane_k >= slot) & (lane_k < slot + n)
                    ktiles[tt] = jnp.where(msk, src, ktiles[tt] if tt in ktiles else zu)

    def prologue(c):
        rows = pl.ds(c * CH, CH)
        qh0 = qh_v[rows, :]
        e0 = jnp.exp2(jnp.dot(jnp.where(gap_r, qh0, 0.0).astype(bf16), build_wk(0, 0),
                              preferred_element_type=f32))
        l0_v[rows, :] = jnp.where(gap_r, qh0, e0)

    def xn_of(c):
        return xn_v[pl.ds(c * CH, CH), :]

    xcps[0].wait()
    for p in range(NPC):
        ln_piece(0, p)
    wq_cp.wait()
    proj_q(0, xn_of(0))
    wv_cp.wait()
    wk_cp.wait()
    wkt_v[...] = wk_v[...].T
    proj_v(0, xn_of(0))
    for c in range(1, NC):
        xcps[c].wait()
    for cp in late:
        cp.start()
    work = [('k', 0), ('p', 0)]
    for c in range(1, NC):
        work += [('v', c), ('k', c), ('q', c), ('p', c)]
    lnq = [(c, p) for c in range(1, NC) for p in range(NPC)]
    for (kind, c) in work:
        per = {'k': NPC, 'p': 0} if c == 0 else {'v': NPC // 2, 'k': NPC - NPC // 2, 'q': 0, 'p': 0}
        for _ in range(per[kind]):
            if lnq and lnq[0][0] == c + 1:
                ln_piece(*lnq.pop(0))
        if kind == 'p':
            prologue(c)
        else:
            {'q': proj_q, 'v': proj_v, 'k': proj_k}[kind](c, xn_of(c))
    for tt in range(16, NT):
        kt_v[tt, 8:328, :] = ktiles[tt]
    for (b, so, n, tt, slot) in PIECES:
        for g in range(NV):
            v_v[g, pl.ds((tt * 128 + slot) // 2, n // 2), :] = v_v[g, pl.ds((b * 128 + so) // 2, n // 2), :]
    w0_v[...] = build_w(0, 0, 0, 1, raw=True)

    lane = _iota((S, 128), 1)

    def fast_epilogue(acc, gapm, chk):
        l = jnp.sum(jnp.where(gapm, 0.0, acc), axis=1, keepdims=True)
        l = jnp.broadcast_to(l, acc.shape)
        rcp = pltpu.reciprocal(l, approx=True)
        o = acc * rcp
        chk = chk + jnp.sum((acc + rcp).reshape(acc.shape[0] // 8, 8, 128), axis=0)
        return o, chk

    def fast_epilogue_chunk(hp, acc_chunk, live, chk, k):
        c, g = head_geom(hp)
        rows = pl.ds(k * RC, RC)
        o, chk = fast_epilogue(acc_chunk, M['gap_c'], chk)
        o = pltpu.roll(o, (c - GP + 128) & 127, 1)
        gd = jnp.where(live, g, NV)
        pltpu.store(attn_v.at[gd, rows, :], o, mask=((lane_c - c) & 127) < DH)
        return chk

    def prep_q_chunk(h, k):
        c, g = head_geom(h)
        return pltpu.roll(q_v[g, pl.ds(k * RC, RC), :], (GP - c + 128) & 127, 1)

    def fast_iter(t, chk):
        zero = jnp.minimum(t, 0)
        gap = lane >= GP + zero
        M['gap_c'] = lane_c >= GP + zero
        M['gap64'] = lane64 >= GP + zero
        M['gap16'] = lane16 >= GP + zero
        M['row16'] = row16 >= 6 + zero
        spare = lane >= 104 + zero
        l0 = l0_v[...]
        q_cur = None
        acc_prev = None
        for u in range(U):
            h = U * t + u
            hnext = jnp.minimum(h + 1, H - 1)
            hprev = jnp.maximum(h - 1, 0)
            lhs = l0.astype(bf16)
            acc = jnp.where(gap, 0.0, l0)
            qn_chunks = []
            q_nxt = None
            for j in range(NT):
                if j == 0 and u == 0:
                    w = pltpu.bitcast(w0_v[...], bf16)
                elif j < NT - 1:
                    w = build_w(h, j, h, j + 1)
                else:
                    w = build_w(h, j, hnext, 0)
                out = jnp.dot(lhs, w, preferred_element_type=f32)
                e = jnp.exp2(out)
                if j < NT - 2:
                    acc = acc + jnp.where(gap, out, e)
                    lhs = jnp.where(gap, qh_v[...] if q_cur is None else q_cur, e).astype(bf16)
                elif j == NT - 2:
                    q_nxt = jnp.concatenate(qn_chunks, axis=0)
                    acc = acc + jnp.where(spare, jnp.where(gap, out, 0.0), e)
                    lhs = jnp.where(gap, q_nxt, e).astype(bf16)
                else:
                    acc = acc + jnp.where(gap, out, 0.0)
                    l0 = jnp.where(gap, q_nxt, e)
                if 1 <= j < 9:
                    k = j - 1
                    ap = acc_v[pl.ds(k * RC, RC), :] if acc_prev is None else acc_prev[k * RC:(k + 1) * RC]
                    chk = fast_epilogue_chunk(hprev, ap, h > 0, chk, k)
                if 9 <= j < 17:
                    k = j - 9
                    qn_chunks.append(prep_q_chunk(hnext, k))
                    if u == U - 1:
                        qh_v[pl.ds(k * RC, RC), :] = qn_chunks[-1]
                if u == U - 1 and j == 16:
                    w0_v[...] = build_w(hnext, 0, hnext, 1, raw=True)
            q_cur = q_nxt
            acc_prev = acc
        l0_v[...] = l0
        acc_v[...] = acc_prev
        return chk

    chk = lax.fori_loop(0, H // U, fast_iter, jnp.zeros((8, 128), f32))
    M.update(M0)

    late[0].wait()
    late[1].wait()
    lane_o = _iota((OCH, 128), 1)
    gap_o = lane_o >= GP
    row8 = _iota((8, 128), 0)

    def orows(c):
        return pl.ds(c * OCH if isinstance(c, int) else pl.multiple_of(c * OCH, OCH), OCH)

    def out_chunk(c, last_o, best, bidx):
        rows = orows(c)
        parts = [attn_v[g, rows, :] for g in range(NG)]
        if last_o is not None:
            parts[NG - 1] = jnp.where(gap_o, last_o, parts[NG - 1])
        for i, hh in enumerate(STRADDLE):
            cc = (DH * hh) % 128
            gg = (DH * hh) // 128
            virt = attn_v[NG + i, rows, :]
            parts[gg] = jnp.where(lane_o >= cc, virt, parts[gg])
            parts[gg + 1] = jnp.where(lane_o < cc + DH - 128, virt, parts[gg + 1])
        lhs = jnp.concatenate(parts, axis=1).astype(bf16)
        hh = x_v[rows, :].astype(f32) + jnp.dot(lhs, wo_v[...], preferred_element_type=f32)
        h_v[rows, :] = hh
        hn = _ln(hh)
        out_v[rows, :] = (hh + hn).astype(bf16)
        hb = hn.astype(bf16).astype(f32)
        wr = wr_v[...].astype(f32)
        pr = hb[:, 0:128] * wr[0:1, :]
        for g in range(1, NG):
            pr = pr + hb[:, g * 128:(g + 1) * 128] * wr[g:g + 1, :]
        r = jnp.sum(pr, axis=1, keepdims=True).astype(bf16).astype(f32)
        r = jnp.broadcast_to(r, (OCH, 128)).reshape(OCH // 8, 8, 128)
        cand = [(r[i], row8 + (c * OCH + i * 8)) for i in range(OCH // 8)]
        while len(cand) > 1:
            nxt = []
            for i in range(0, len(cand), 2):
                (va, ia), (vb, ib) = cand[i], cand[i + 1]
                upd = vb > va
                nxt.append((jnp.where(upd, vb, va), jnp.where(upd, ib, ia)))
            cand = nxt
        upd = cand[0][0] > best
        return jnp.where(upd, cand[0][0], best), jnp.where(upd, cand[0][1], bidx)

    def out_copy(c):
        return pltpu.make_async_copy(out_v.at[orows(c), :], out_hbm.at[orows(c), :], osems.at[c])

    best = jnp.full((8, 128), -jnp.inf, f32)
    bidx = jnp.zeros((8, 128), jnp.int32)
    for c in range(S // OCH):
        last_o, chk = fast_epilogue(acc_v[orows(c), :], gap_o, chk)
        best, bidx = out_chunk(c, last_o, best, bidx)
        out_copy(c).start()
    top_v[0] = best
    top_v[1] = bidx.astype(f32)
    ok = jnp.max(jnp.where(jnp.abs(chk) < GUARD, 0, 1)) == 0

    @pl.when(jnp.logical_not(ok))
    def _():
        for c in range(S // OCH):
            out_copy(c).wait()
        lane_s = _iota((CH, 128), 1)
        gap_s = lane_s >= GP

        def safe_head(h, carry):
            c, g = head_geom(h)

            def rows_body(r, c2):
                rows = pl.ds(pl.multiple_of(r * CH, CH), CH)
                qh = pltpu.roll(q_v[g, rows, :], (GP - c + 128) & 127, 1)
                lq = jnp.where(gap_s, qh, 0.0).astype(bf16)

                def valid(j):
                    return (lane_s < GP) & ((j < NT - 1) | (lane_s < 104))

                def max_body(j, m):
                    s = jnp.dot(lq, build_wk(h, j), preferred_element_type=f32)
                    s = jnp.where(valid(j), s, -jnp.inf)
                    return jnp.maximum(m, jnp.max(s, axis=1, keepdims=True))
                m = lax.fori_loop(0, NT, max_body, jnp.full((CH, 1), -jnp.inf, f32))

                def pv_body(j, acc):
                    s = jnp.dot(lq, build_wk(h, j), preferred_element_type=f32)
                    p = jnp.where(valid(j), jnp.exp2(s - m), 0.0)
                    o = jnp.dot(p.astype(bf16), build_wv(h, j), preferred_element_type=f32)
                    return acc + jnp.where(gap_s, o, p)
                acc = lax.fori_loop(0, NT, pv_body, jnp.zeros((CH, 128), f32))
                l = jnp.sum(jnp.where(gap_s, 0.0, acc), axis=1, keepdims=True)
                o = pltpu.roll(acc * (1.0 / l), (c - GP + 128) & 127, 1)
                pltpu.store(attn_v.at[g, rows, :], o, mask=((lane_s - c) & 127) < DH)
                return c2
            lax.fori_loop(0, S // CH, rows_body, 0)
            return carry

        lax.fori_loop(0, H, safe_head, 0)

        def redo_chunk(c, carry):
            b2, i2 = out_chunk(c, None, carry[0], carry[1])
            out_copy(c).start()
            return b2, i2
        b2, i2 = lax.fori_loop(0, S // OCH, redo_chunk,
                               (jnp.full((8, 128), -jnp.inf, f32), jnp.zeros((8, 128), jnp.int32)))
        top_v[0] = b2
        top_v[1] = i2.astype(f32)

    best = top_v[0]
    rmax = jnp.max(best)
    sel = jnp.min(jnp.where(best == rmax, top_v[1], float(S - 1))).astype(jnp.int32)

    late[2].wait()
    late[3].wait()
    late[4].wait()
    hrow = h_v[pl.ds(sel, 1), :]
    hnrow = _ln(hrow)
    xs = jnp.broadcast_to(hnrow, (16, D)).astype(bf16)
    gg = jnp.dot(xs, wg_v[...], preferred_element_type=f32)
    uu = jnp.dot(xs, wu_v[...], preferred_element_type=f32)
    act = (gg * jax.nn.sigmoid(gg) * uu).astype(bf16)
    yy = jnp.dot(act, wd_v[...], preferred_element_type=f32)
    yy = yy * jax.nn.sigmoid(jnp.full((16, D), rmax, f32))
    base = pl.multiple_of((sel // 16) * 16, 16)
    new = (jnp.broadcast_to(hrow + hnrow, (16, D)) + yy).astype(bf16)
    patch_v[...] = jnp.where(_iota((16, D), 0) == sel - base, new, out_v[pl.ds(base, 16), :])
    for c in range(S // OCH):
        out_copy(c).wait()
    cp = pltpu.make_async_copy(patch_v, out_hbm.at[pl.ds(base, 16), :], osems.at[0])
    cp.start()
    cp.wait()


@jax.jit
def pallas_sequential_preLN__mha_block__moe_arch_mod__prompt_kernel(
    A_x: jax.Array,
    A_wqkv: jax.Array,
    A_wo: jax.Array,
    B_x: jax.Array,
    B_w_r: jax.Array,
    B_w_gate: jax.Array,
    B_w_up: jax.Array,
    B_w_down: jax.Array,
):
    del B_x
    any_spec = pl.BlockSpec(memory_space=pl.ANY)
    scratch = [
        pltpu.VMEM((S, D), bf16),
        pltpu.VMEM((S, D), bf16),
        pltpu.VMEM((D, D), bf16),
        pltpu.VMEM((D, D), bf16),
        pltpu.VMEM((D, D), bf16),
        pltpu.VMEM((D, D), bf16),
        pltpu.VMEM((D, D), bf16),
        pltpu.VMEM((NG, 128), bf16),
        pltpu.VMEM((D, F), bf16),
        pltpu.VMEM((D, F), bf16),
        pltpu.VMEM((F, D), bf16),
        pltpu.VMEM((NV, S, 128), f32),
        pltpu.VMEM((NV, NT * 64, 128), u32),
        pltpu.VMEM((NT, KTR, 128), u32),
        pltpu.VMEM((S, 128), f32),
        pltpu.VMEM((S, 128), f32),
        pltpu.VMEM((S, 128), f32),
        pltpu.VMEM((64, 128), u32),
        pltpu.VMEM((NV + 1, S, 128), f32),
        pltpu.VMEM((S, D), f32),
        pltpu.VMEM((S, D), bf16),
        pltpu.VMEM((16, D), bf16),
        pltpu.VMEM((2, 8, 128), f32),
        pltpu.SemaphoreType.DMA((S // CH + 8,)),
        pltpu.SemaphoreType.DMA((S // OCH,)),
    ]
    out = pl.pallas_call(
        _kernel,
        out_shape=jax.ShapeDtypeStruct((S, D), bf16),
        in_specs=[any_spec] * 7,
        out_specs=any_spec,
        scratch_shapes=scratch,
        compiler_params=pltpu.CompilerParams(vmem_limit_bytes=127 * 1024 * 1024),
    )(A_x.reshape(S, D), A_wqkv, A_wo, B_w_r.reshape(NG, 128), B_w_gate, B_w_up, B_w_down)
    return out.reshape(1, S, D)
```
